```python
import jax
import jax.numpy as jnp

def _softmax(x, axis=-1):
    return jax.nn.softmax(x, axis=axis)

def _gelu(x):
    return jax.nn.gelu(x, approximate=True)

def _silu(x):
    return jax.nn.silu(x)

def _sigmoid(x):
    return jax.nn.sigmoid(x)

def _layernorm(x, axis=-1, eps=1e-05):
    m = jnp.mean(x, axis=axis, keepdims=True)
    v = jnp.var(x, axis=axis, keepdims=True)
    return (x - m) / jnp.sqrt(v + eps)

def _scatter_add(tgt, idx, src, axis=0):
    return tgt.at[idx].add(src)

def _segment_sum(src, seg, n):
    return jax.ops.segment_sum(src, seg, n)

class _Rng:

    def __init__(self, key):
        self._k = key

    def _next(self):
        self._k, sub = jax.random.split(self._k)
        return sub

    def normal(self, shape):
        return jax.random.normal(self._next(), shape, dtype=jnp.bfloat16)

    def randint(self, lo, hi, shape):
        return jax.random.randint(self._next(), shape, lo, hi, dtype=jnp.int32)

    def uniform(self, shape, lo=0.0, hi=1.0):
        return jax.random.uniform(self._next(), shape, jnp.bfloat16, lo, hi)

    def permutation(self, n):
        return jax.random.permutation(self._next(), n)
kernel_name = 'adaLN_cond__sliding_block_cached__glu_gated_glu__decode'

def setup_inputs():
    _rng = _Rng(jax.random.key(int.from_bytes(__import__("os").urandom(4), "little")))
    _w = lambda a: (lambda t: t.astype(jnp.bfloat16) if jnp.issubdtype(t.dtype, jnp.floating) else t)(jnp.asarray(a))

    def _A_setup():
        B, Sq, D = (8, 1, 512)
        Hq, Hkv, Sk, Dh = (32, 32, 4096, 128)
        assert Hq % Hkv == 0, (Hq, Hkv)
        return {'x': _w((lambda *s: _rng.normal(s) * 0.05)(B, Sq, D)), 'k_cache': _w((lambda *s: _rng.normal(s) * 0.05)(B, Hkv, Sk, Dh)), 'v_cache': _w((lambda *s: _rng.normal(s) * 0.05)(B, Hkv, Sk, Dh)), 'wq': _w((lambda *s: _rng.normal(s) * 0.05)(D, Hq * Dh) * D ** (-0.5)), 'wo': _w((lambda *s: _rng.normal(s) * 0.05)(Hq * Dh, D) * (Hq * Dh) ** (-0.5))}
    _A_in = _A_setup()

    def _B_setup():
        B, S, D, F = (8, 1, 512, 1376)
        return {'x': _w((lambda *s: _rng.normal(s) * 0.05)(B, S, D)), 'w_gate': _w((lambda *s: _rng.normal(s) * 0.05)(D, F)), 'w_up': _w((lambda *s: _rng.normal(s) * 0.05)(D, F)), 'w_down': _w((lambda *s: _rng.normal(s) * 0.05)(F, D))}
    _B_in = _B_setup()
    return {'A_x': _A_in['x'], 'A_k_cache': _A_in['k_cache'], 'A_v_cache': _A_in['v_cache'], 'A_wq': _A_in['wq'], 'A_wo': _A_in['wo'], 'B_x': _B_in['x'], 'B_w_gate': _B_in['w_gate'], 'B_w_up': _B_in['w_up'], 'B_w_down': _B_in['w_down'], 'c': _w((lambda *s: _rng.normal(s) * 0.05)(8, 512)), 'w_mod': _w((lambda *s: _rng.normal(s) * 0.05)(512, 6 * 512) * 512 ** (-0.5))}

def reference(A_x, A_k_cache, A_v_cache, A_wq, A_wo, B_x, B_w_gate, B_w_up, B_w_down, c, w_mod):

    def _A_ref(x, k_cache, v_cache, wq, wo):
        B, Sq, D = x.shape
        Hq, Dh = (32, 128)
        Hkv, Sk = (k_cache.shape[1], k_cache.shape[2])
        W = min(4096, max(256, Sk // 4))
        rep = Hq // Hkv
        q = (lambda x, *d: x.transpose(*d))((x @ wq).reshape(B, Sq, Hq, Dh), 0, 2, 1, 3)
        k = jnp.repeat(k_cache[:, :, Sk - W:, :], rep, axis=1)
        v = jnp.repeat(v_cache[:, :, Sk - W:, :], rep, axis=1)
        scores = jnp.einsum('bhqd,bhkd->bhqk', q, k) * Dh ** (-0.5)
        p = _softmax(scores, axis=-1)
        o = jnp.einsum('bhqk,bhkd->bhqd', p, v)
        return (lambda x, *d: x.transpose(*d))(o, 0, 2, 1, 3).reshape(B, Sq, Hq * Dh) @ wo

    def _B_ref(x, w_gate, w_up, w_down):
        g = jnp.einsum('bsd,df->bsf', x, w_gate)
        u = jnp.einsum('bsd,df->bsf', x, w_up)
        h = _sigmoid(g) * u
        return jnp.einsum('bsf,fd->bsd', h, w_down)
    x = A_x
    mod = (_silu(c) @ w_mod).reshape(c.shape[0], 6, 1, -1)
    sa, ca, ga, sb, cb, gb = (mod[:, 0].copy(), mod[:, 1].copy(), mod[:, 2].copy(), mod[:, 3].copy(), mod[:, 4].copy(), mod[:, 5].copy())
    h = _layernorm(x, axis=-1) * (1 + ca) + sa
    x = x + ga * _A_ref(h, A_k_cache, A_v_cache, A_wq, A_wo)
    h = _layernorm(x, axis=-1) * (1 + cb) + sb
    x = x + gb * _B_ref(h, B_w_gate, B_w_up, B_w_down)
    return x
```

```python
import functools

import jax
import jax.numpy as jnp
import jax.experimental.pallas as pl
import jax.experimental.pallas.tpu as pltpu

_HQ = 32
_DH = 128
_HG = 4
_ROWS = 32
_NBUF = 4
_EPS = 1e-5


def _layernorm(x):
    m = jnp.mean(x, axis=-1, keepdims=True)
    xc = x - m
    v = jnp.mean(xc * xc, axis=-1, keepdims=True)
    return xc * jax.lax.rsqrt(v + _EPS)


def _sigmoid(x):
    return 1.0 / (1.0 + jnp.exp(-x))


def _kernel(x_ref, c_ref, k_hbm, v_hbm, wq_hbm, wo_hbm, wg_hbm, wu_hbm, wd_hbm, wmod_hbm,
            o_ref,
            kbuf, vbuf, wq_buf, wo_buf, wg_buf, wu_buf, wd_buf, wmod_buf,
            q_scr, oh_scr, kv_sem, w_sem, *, B, D, Sk, W):
    n_units = B * (_HQ // _HG)
    n_pieces = W // _ROWS
    f32, bf16 = jnp.float32, jnp.bfloat16

    def start_unit(u, slot):
        hg = u // B
        b = u % B

        def one(r, carry):
            r0 = pl.multiple_of(r * _ROWS, _ROWS)
            pltpu.make_async_copy(
                k_hbm.at[b, pl.ds(hg * _HG, _HG), pl.ds(Sk - W + r0, _ROWS), :],
                kbuf.at[slot, :, pl.ds(r0, _ROWS), :], kv_sem.at[0, slot]).start(priority=0)
            pltpu.make_async_copy(
                v_hbm.at[b, pl.ds(hg * _HG, _HG), pl.ds(Sk - W + r0, _ROWS), :],
                vbuf.at[slot, :, pl.ds(r0, _ROWS), :], kv_sem.at[1, slot]).start(priority=1)
            return carry

        jax.lax.fori_loop(0, n_pieces, one, 0)

    w_pairs = ((wmod_hbm, wmod_buf), (wq_hbm, wq_buf), (wo_hbm, wo_buf),
               (wg_hbm, wg_buf), (wu_hbm, wu_buf), (wd_hbm, wd_buf))
    w_copies = [pltpu.make_async_copy(s, d, w_sem.at[i]) for i, (s, d) in enumerate(w_pairs)]

    w_copies[0].start(priority=0)
    w_copies[1].start(priority=1)
    for u in range(_NBUF - 1):
        start_unit(u, u)
    for i in range(2, 6):
        w_copies[i].start(priority=i % 2)

    x = x_ref[...].astype(f32)
    c = c_ref[...].astype(f32)
    sc = (c * _sigmoid(c)).astype(bf16)
    w_copies[0].wait()
    mod = jnp.dot(sc, wmod_buf[...], preferred_element_type=f32)
    sa, ca, ga, sb, cb, gb = (mod[:, i * D:(i + 1) * D] for i in range(6))
    h = (_layernorm(x) * (1.0 + ca) + sa).astype(bf16)
    w_copies[1].wait()
    q = jnp.dot(h, wq_buf[...], preferred_element_type=f32)
    for hh in range(_HQ):
        q_scr[hh] = q[:, hh * _DH:(hh + 1) * _DH]
    oh_scr[...] = jnp.zeros(oh_scr.shape, f32)

    scale = _DH ** -0.5
    row = jax.lax.broadcasted_iota(jnp.int32, (B, _DH), 0)

    def body(u, carry):
        slot = u % _NBUF
        nxt = u + _NBUF - 1

        @pl.when(nxt < n_units)
        def _():
            start_unit(nxt, nxt % _NBUF)

        hg = u // B
        b = u % B
        pltpu.make_async_copy(kbuf.at[slot], kbuf.at[slot], kv_sem.at[0, slot]).wait()
        pltpu.make_async_copy(vbuf.at[slot], vbuf.at[slot], kv_sem.at[1, slot]).wait()
        for j in range(_HG):
            hh = hg * _HG + j
            qh = q_scr[hh].astype(bf16)
            s = jax.lax.dot_general(qh, kbuf[slot, j], (((1,), (1,)), ((), ())),
                                    preferred_element_type=f32)
            m = jnp.max(s, axis=-1, keepdims=True)
            p = jnp.exp((s - m) * scale)
            l = jnp.sum(p, axis=-1, keepdims=True)
            o = jnp.dot(p.astype(bf16), vbuf[slot, j], preferred_element_type=f32)
            o = o / l
            oh_scr[hh] = jnp.where(row == b, o, oh_scr[hh])
        return carry

    jax.lax.fori_loop(0, n_units, body, 0)

    o_all = jnp.concatenate([oh_scr[hh] for hh in range(_HQ)], axis=-1).astype(bf16)
    w_copies[2].wait()
    attn = jnp.dot(o_all, wo_buf[...], preferred_element_type=f32)
    x1 = x + ga * attn
    h2 = (_layernorm(x1) * (1.0 + cb) + sb).astype(bf16)
    w_copies[3].wait()
    nt = (((1,), (1,)), ((), ()))
    g = jax.lax.dot_general(h2, wg_buf[...], nt, preferred_element_type=f32)
    w_copies[4].wait()
    up = jax.lax.dot_general(h2, wu_buf[...], nt, preferred_element_type=f32)
    hid = (_sigmoid(g) * up).astype(bf16)
    w_copies[5].wait()
    y = jnp.dot(hid, wd_buf[...], preferred_element_type=f32)
    o_ref[...] = (x1 + gb * y).astype(o_ref.dtype)


@jax.jit
def pallas_adaLN_cond__sliding_block_cached__glu_gated_glu__decode_kernel(
    A_x: jax.Array,
    A_k_cache: jax.Array,
    A_v_cache: jax.Array,
    A_wq: jax.Array,
    A_wo: jax.Array,
    B_x: jax.Array,
    B_w_gate: jax.Array,
    B_w_up: jax.Array,
    B_w_down: jax.Array,
    c: jax.Array,
    w_mod: jax.Array,
):
    B, Sq, D = A_x.shape
    _, Hkv, Sk, Dh = A_k_cache.shape
    assert Sq == 1 and Hkv == _HQ and Dh == _DH
    W = min(4096, max(256, Sk // 4))
    bf16 = jnp.bfloat16

    any_spec = pl.BlockSpec(memory_space=pltpu.MemorySpace.HBM)
    vmem_spec = pl.BlockSpec(memory_space=pltpu.VMEM)
    out = pl.pallas_call(
        functools.partial(_kernel, B=B, D=D, Sk=Sk, W=W),
        out_shape=jax.ShapeDtypeStruct((B, D), A_x.dtype),
        in_specs=[vmem_spec, vmem_spec] + [any_spec] * 8,
        out_specs=vmem_spec,
        scratch_shapes=[
            pltpu.VMEM((_NBUF, _HG, W, _DH), bf16),
            pltpu.VMEM((_NBUF, _HG, W, _DH), bf16),
            pltpu.VMEM(A_wq.shape, bf16),
            pltpu.VMEM(A_wo.shape, bf16),
            pltpu.VMEM(B_w_down.shape, bf16),
            pltpu.VMEM(B_w_down.shape, bf16),
            pltpu.VMEM(B_w_down.shape, bf16),
            pltpu.VMEM(w_mod.shape, bf16),
            pltpu.VMEM((_HQ, B, _DH), jnp.float32),
            pltpu.VMEM((_HQ, B, _DH), jnp.float32),
            pltpu.SemaphoreType.DMA((2, _NBUF)),
            pltpu.SemaphoreType.DMA((6,)),
        ],
        compiler_params=pltpu.CompilerParams(vmem_limit_bytes=100 * 1024 * 1024,
                                             disable_bounds_checks=True),
    )(A_x.reshape(B, D), c, A_k_cache, A_v_cache, A_wq, A_wo, B_w_gate.T, B_w_up.T, B_w_down, w_mod)
    return out.reshape(B, Sq, D)
```

```python
import functools

import jax
import jax.numpy as jnp
import jax.experimental.pallas as pl
import jax.experimental.pallas.tpu as pltpu

_HQ = 32
_DH = 128
_HU = 16
_NHI = 2
_ROWS = 16
_NSUB = 2
_EPS = 1e-5


def _layernorm(x):
    m = jnp.mean(x, axis=-1, keepdims=True)
    xc = x - m
    v = jnp.mean(xc * xc, axis=-1, keepdims=True)
    return xc * jax.lax.rsqrt(v + _EPS)


def _sigmoid(x):
    return 1.0 / (1.0 + jnp.exp(-x))


def _kernel(x_hbm, c_hbm, k_hbm, v_hbm, wq_hbm, wo_hbm, wg_hbm, wu_hbm, wd_hbm, wmod_hbm,
            o_ref,
            kbuf, vbuf, wq_buf, wo_buf, wg_buf, wu_buf, wd_buf, wmod_buf, x_buf, c_buf,
            q_scr, p_scr, oh_scr, kv_sem, w_sem, *, B, D, F, Sk, W):
    upb = _HQ // _HU
    n_units = B * upb
    n_blk = W // _ROWS // _NSUB
    hps = _HU // _NSUB
    f32, bf16 = jnp.float32, jnp.bfloat16
    nt = (((1,), (1,)), ((), ()))
    S_X, S_C, S_MOD, S_Q, S_O, S_G, S_U, S_D = range(8)

    def copy(src, dst, sem, prio):
        pltpu.make_async_copy(src, dst, sem).start(priority=prio)

    def wait_all(buf, sem):
        pltpu.make_async_copy(buf, buf, sem).wait()

    def issue_kv(a, u, sub):
        src, dst = ((k_hbm, kbuf), (v_hbm, vbuf))[a]
        slot = u % 2
        b = u // upb
        h0 = (u % upb) * _HU

        def one(r, carry):
            r0 = pl.multiple_of((sub * n_blk + r) * _ROWS, _ROWS)
            rows_s, rows_d = pl.ds(Sk - W + r0, _ROWS), pl.ds(r0, _ROWS)
            copy(src.at[b, pl.ds(h0, _NHI), rows_s, :],
                 dst.at[slot, pl.ds(0, _NHI), rows_d, :], kv_sem.at[a, slot], 0)
            copy(src.at[b, pl.ds(h0 + _NHI, _HU - _NHI), rows_s, :],
                 dst.at[slot, pl.ds(_NHI, _HU - _NHI), rows_d, :], kv_sem.at[a, slot], 1)
            return carry

        jax.lax.fori_loop(0, n_blk, one, 0, unroll=4)

    prio4 = (0, 1, 1, 1)

    def issue_head():
        rs = D // 4

        def one(j, carry):
            r = pl.multiple_of((j // 2) * 8, 8)
            half = j % 2
            cm = pl.multiple_of(half * (3 * D), 128)
            cq = pl.multiple_of(half * (_HQ * _DH // 2), 128)
            for g in range(4):
                rows = pl.ds(g * rs + r, 8)
                cols = pl.ds(cm, 3 * D)
                copy(wmod_hbm.at[rows, cols], wmod_buf.at[rows, cols], w_sem.at[S_MOD], prio4[(2 * g) % 4])
                cols = pl.ds(cq, _HQ * _DH // 2)
                copy(wq_hbm.at[rows, cols], wq_buf.at[rows, cols], w_sem.at[S_Q], prio4[(2 * g + 1) % 4])
            return carry

        jax.lax.fori_loop(0, 2 * rs // 8, one, 0)

    def issue_wo(sub):
        rs = _HQ * _DH // 8
        n = rs // 32 // _NSUB

        def one(j, carry):
            r = pl.multiple_of((sub * n + j) * 32, 32)
            for g in range(8):
                rows = pl.ds(g * rs + r, 32)
                copy(wo_hbm.at[rows], wo_buf.at[rows], w_sem.at[S_O], prio4[g % 4])
            return carry

        jax.lax.fori_loop(0, n, one, 0)

    n_fp = F // 32
    perm = [(j * 11) % n_fp for j in range(n_fp)]
    ffn_list = []
    for j in perm:
        ffn_list.append((wg_hbm, wg_buf, S_G, j))
        ffn_list.append((wu_hbm, wu_buf, S_U, j))
    for j in perm:
        ffn_list.append((wd_hbm, wd_buf, S_D, j))

    def issue_ffn(sub):
        n = len(ffn_list)
        lo, hi = sub * n // _NSUB, (sub + 1) * n // _NSUB
        for idx in range(lo, hi):
            src, dst, s, j = ffn_list[idx]
            rows = pl.ds(j * 32, 32)
            copy(src.at[rows], dst.at[rows], w_sem.at[s], prio4[idx % 4])

    copy(x_hbm, x_buf, w_sem.at[S_X], 0)
    copy(c_hbm, c_buf, w_sem.at[S_C], 0)
    issue_head()
    for sub in range(_NSUB):
        issue_kv(0, 0, sub)

    wait_all(x_buf, w_sem.at[S_X])
    wait_all(c_buf, w_sem.at[S_C])
    x = x_buf[...].astype(f32)
    c = c_buf[...].astype(f32)
    sc = (c * _sigmoid(c)).astype(bf16)
    wait_all(wmod_buf, w_sem.at[S_MOD])
    mod = jnp.dot(sc, wmod_buf[...], preferred_element_type=f32)
    sa, ca, ga, sb, cb, gb = (mod[:, i * D:(i + 1) * D] for i in range(6))
    h = (_layernorm(x) * (1.0 + ca) + sa).astype(bf16)
    issue_kv(1, 0, 0)
    wait_all(wq_buf, w_sem.at[S_Q])
    q = jnp.dot(h, wq_buf[...], preferred_element_type=f32)
    for hh in range(_HQ):
        q_scr[hh] = q[:, hh * _DH:(hh + 1) * _DH]
    oh_scr[...] = jnp.zeros(oh_scr.shape, f32)
    for sub in range(1, _NSUB):
        issue_kv(1, 0, sub)

    scale = _DH ** -0.5
    row = jax.lax.broadcasted_iota(jnp.int32, (B, _DH), 0)

    def body(u, carry):
        slot = u % 2
        b = u // upb
        h0 = (u % upb) * _HU
        more = u + 1 < n_units

        for sub in range(_NSUB):
            @pl.when(more)
            def _():
                issue_kv(0, u + 1, sub)

            @pl.when(jnp.logical_not(more))
            def _():
                issue_wo(sub)

            if sub == 0:
                wait_all(kbuf.at[slot], kv_sem.at[0, slot])
            for j in range(sub * hps, (sub + 1) * hps):
                qh = q_scr[h0 + j].astype(bf16)
                s = jax.lax.dot_general(qh, kbuf[slot, j], nt, preferred_element_type=f32)
                m = jnp.max(s, axis=-1, keepdims=True)
                e = jnp.exp((s - m) * scale)
                l = jnp.sum(e, axis=-1, keepdims=True)
                p_scr[j] = e * (1.0 / l)

        for sub in range(_NSUB):
            @pl.when(more)
            def _():
                issue_kv(1, u + 1, sub)

            @pl.when(jnp.logical_not(more))
            def _():
                issue_ffn(sub)

            if sub == 0:
                wait_all(vbuf.at[slot], kv_sem.at[1, slot])
            for j in range(sub * hps, (sub + 1) * hps):
                o = jnp.dot(p_scr[j].astype(bf16), vbuf[slot, j], preferred_element_type=f32)
                oh_scr[h0 + j] = jnp.where(row == b, o, oh_scr[h0 + j])
        return carry

    jax.lax.fori_loop(0, n_units, body, 0)

    o_all = jnp.concatenate([oh_scr[hh] for hh in range(_HQ)], axis=-1).astype(bf16)
    wait_all(wo_buf, w_sem.at[S_O])
    attn = jnp.dot(o_all, wo_buf[...], preferred_element_type=f32)
    x1 = x + ga * attn
    h2 = (_layernorm(x1) * (1.0 + cb) + sb).astype(bf16)
    wait_all(wg_buf, w_sem.at[S_G])
    g = jax.lax.dot_general(h2, wg_buf[...], nt, preferred_element_type=f32)
    wait_all(wu_buf, w_sem.at[S_U])
    up = jax.lax.dot_general(h2, wu_buf[...], nt, preferred_element_type=f32)
    hid = (_sigmoid(g) * up).astype(bf16)
    wait_all(wd_buf, w_sem.at[S_D])
    y = jnp.dot(hid, wd_buf[...], preferred_element_type=f32)
    o_ref[...] = (x1 + gb * y).astype(o_ref.dtype)


@jax.jit
def pallas_adaLN_cond__sliding_block_cached__glu_gated_glu__decode_kernel(
    A_x: jax.Array,
    A_k_cache: jax.Array,
    A_v_cache: jax.Array,
    A_wq: jax.Array,
    A_wo: jax.Array,
    B_x: jax.Array,
    B_w_gate: jax.Array,
    B_w_up: jax.Array,
    B_w_down: jax.Array,
    c: jax.Array,
    w_mod: jax.Array,
):
    B, Sq, D = A_x.shape
    _, Hkv, Sk, Dh = A_k_cache.shape
    F = B_w_down.shape[0]
    assert Sq == 1 and Hkv == _HQ and Dh == _DH
    W = min(4096, max(256, Sk // 4))
    bf16 = jnp.bfloat16

    hbm_spec = pl.BlockSpec(memory_space=pltpu.MemorySpace.HBM)
    out = pl.pallas_call(
        functools.partial(_kernel, B=B, D=D, F=F, Sk=Sk, W=W),
        out_shape=jax.ShapeDtypeStruct((B, D), A_x.dtype),
        in_specs=[hbm_spec] * 10,
        out_specs=pl.BlockSpec(memory_space=pltpu.VMEM),
        scratch_shapes=[
            pltpu.VMEM((2, _HU, W, _DH), bf16),
            pltpu.VMEM((2, _HU, W, _DH), bf16),
            pltpu.VMEM(A_wq.shape, bf16),
            pltpu.VMEM(A_wo.shape, bf16),
            pltpu.VMEM((F, D), bf16),
            pltpu.VMEM((F, D), bf16),
            pltpu.VMEM((F, D), bf16),
            pltpu.VMEM(w_mod.shape, bf16),
            pltpu.VMEM((B, D), bf16),
            pltpu.VMEM((B, D), bf16),
            pltpu.VMEM((_HQ, B, _DH), jnp.float32),
            pltpu.VMEM((_HU, B, W), jnp.float32),
            pltpu.VMEM((_HQ, B, _DH), jnp.float32),
            pltpu.SemaphoreType.DMA((2, 2)),
            pltpu.SemaphoreType.DMA((8,)),
        ],
        compiler_params=pltpu.CompilerParams(vmem_limit_bytes=64 * 1024 * 1024,
                                             disable_bounds_checks=True),
    )(A_x.reshape(B, D), c, A_k_cache, A_v_cache, A_wq, A_wo, B_w_gate.T, B_w_up.T, B_w_down, w_mod)
    return out.reshape(B, Sq, D)
```

```python
import functools

import jax
import jax.numpy as jnp
import jax.experimental.pallas as pl
import jax.experimental.pallas.tpu as pltpu

_HQ = 32
_DH = 128
_HU = 16
_NHI = 2
_ROWS = 16
_NSUB = 2
_WD_SPLIT = (128, 384)
_LO_LAG = 32
_FFN_CUT = (64, 96)
_EPS = 1e-5


def _layernorm(x):
    m = jnp.mean(x, axis=-1, keepdims=True)
    xc = x - m
    v = jnp.mean(xc * xc, axis=-1, keepdims=True)
    return xc * jax.lax.rsqrt(v + _EPS)


def _sigmoid(x):
    return 1.0 / (1.0 + jnp.exp(-x))


def _kernel(x_hbm, c_hbm, k_hbm, v_hbm, wq_hbm, wo_hbm, wg_hbm, wu_hbm, wd_hbm, wmod_hbm,
            o_ref,
            kbuf, vbuf, wq_buf, wo_buf, wg_buf, wu_buf, wd_buf, wmod_buf, x_buf, c_buf,
            q_scr, p_scr, oh_scr, kv_sem, w_sem, *, B, D, F, Sk, W):
    upb = _HQ // _HU
    n_units = B * upb
    n_blk = W // _ROWS // _NSUB
    hps = _HU // _NSUB
    f32, bf16 = jnp.float32, jnp.bfloat16
    nt = (((1,), (1,)), ((), ()))
    S_X, S_C, S_MOD, S_Q, S_O, S_G, S_U, S_D, S_D1, S_D2 = range(10)

    def copy(src, dst, sem, prio):
        pltpu.make_async_copy(src, dst, sem).start(priority=prio)

    def wait_all(buf, sem):
        pltpu.make_async_copy(buf, buf, sem).wait()

    def issue_kv(a, u, sub):
        src, dst = ((k_hbm, kbuf), (v_hbm, vbuf))[a]
        slot = u % 2
        b = u // upb
        h0 = (u % upb) * _HU

        def one(r, carry):
            r0 = pl.multiple_of((sub * n_blk + r) * _ROWS, _ROWS)
            rows_s, rows_d = pl.ds(Sk - W + r0, _ROWS), pl.ds(r0, _ROWS)
            copy(src.at[b, pl.ds(h0, _NHI), rows_s, :],
                 dst.at[slot, pl.ds(0, _NHI), rows_d, :], kv_sem.at[a, slot], 0)
            copy(src.at[b, pl.ds(h0 + _NHI, _HU - _NHI), rows_s, :],
                 dst.at[slot, pl.ds(_NHI, _HU - _NHI), rows_d, :], kv_sem.at[a, slot], 1)
            return carry

        jax.lax.fori_loop(0, n_blk, one, 0, unroll=4)

    prio4 = (0, 1, 1, 1)

    def issue_head():
        rs = D // 4

        def one(j, carry):
            r = pl.multiple_of((j // 2) * 8, 8)
            half = j % 2
            cm = pl.multiple_of(half * (3 * D), 128)
            cq = pl.multiple_of(half * (_HQ * _DH // 2), 128)
            for g in range(4):
                rows = pl.ds(g * rs + r, 8)
                cols = pl.ds(cm, 3 * D)
                copy(wmod_hbm.at[rows, cols], wmod_buf.at[rows, cols], w_sem.at[S_MOD], prio4[(2 * g) % 4])
                cols = pl.ds(cq, _HQ * _DH // 2)
                copy(wq_hbm.at[rows, cols], wq_buf.at[rows, cols], w_sem.at[S_Q], prio4[(2 * g + 1) % 4])
            return carry

        jax.lax.fori_loop(0, 2 * rs // 8, one, 0)

    def issue_wo(sub):
        rs = _HQ * _DH // 8
        n = rs // 32 // _NSUB

        def one(j, carry):
            r = pl.multiple_of((sub * n + j) * 32, 32)
            for g in range(8):
                rows = pl.ds(g * rs + r, 32)
                copy(wo_hbm.at[rows], wo_buf.at[rows], w_sem.at[S_O], prio4[g % 4])
            return carry

        jax.lax.fori_loop(0, n, one, 0)

    n_fp = F // 32
    perm = [(j * 11) % n_fp for j in range(n_fp)]
    d1, d2 = _WD_SPLIT
    done_order = [(wg_hbm, wg_buf, S_G, j) for j in perm]
    done_order += [(wu_hbm, wu_buf, S_U, j) for j in perm]
    done_order += [(wd_hbm, wd_buf, S_D, j) for j in perm if j * 32 >= d2]
    done_order += [(wd_hbm, wd_buf, S_D1, j) for j in range(d1 // 32, d2 // 32)]
    done_order += [(wd_hbm, wd_buf, S_D2, j) for j in range(d1 // 32)]
    n_ffn = len(done_order)
    slots = sorted(range(n_ffn), key=lambda t: t + _LO_LAG * prio4[t % 4])
    ffn_list = [None] * n_ffn
    for piece, t in zip(done_order, slots):
        ffn_list[t] = piece

    def issue_ffn(lo, hi):
        for idx in range(lo, min(hi, n_ffn)):
            src, dst, s, j = ffn_list[idx]
            rows = pl.ds(j * 32, 32)
            copy(src.at[rows], dst.at[rows], w_sem.at[s], prio4[idx % 4])

    copy(x_hbm, x_buf, w_sem.at[S_X], 0)
    copy(c_hbm, c_buf, w_sem.at[S_C], 0)
    issue_head()
    for sub in range(_NSUB):
        issue_kv(0, 0, sub)

    wait_all(x_buf, w_sem.at[S_X])
    wait_all(c_buf, w_sem.at[S_C])
    x = x_buf[...].astype(f32)
    c = c_buf[...].astype(f32)
    sc = (c * _sigmoid(c)).astype(bf16)
    wait_all(wmod_buf, w_sem.at[S_MOD])
    mod = jnp.dot(sc, wmod_buf[...], preferred_element_type=f32)
    sa, ca, ga, sb, cb, gb = (mod[:, i * D:(i + 1) * D] for i in range(6))
    h = (_layernorm(x) * (1.0 + ca) + sa).astype(bf16)
    issue_kv(1, 0, 0)
    wait_all(wq_buf, w_sem.at[S_Q])
    q = jnp.dot(h, wq_buf[...], preferred_element_type=f32)
    for hh in range(_HQ):
        q_scr[hh] = q[:, hh * _DH:(hh + 1) * _DH]
    oh_scr[...] = jnp.zeros(oh_scr.shape, f32)
    for sub in range(1, _NSUB):
        issue_kv(1, 0, sub)

    scale = _DH ** -0.5
    row = jax.lax.broadcasted_iota(jnp.int32, (B, _DH), 0)

    def body(u, carry):
        slot = u % 2
        b = u // upb
        h0 = (u % upb) * _HU
        more = u + 1 < n_units

        for sub in range(_NSUB):
            @pl.when(more)
            def _():
                issue_kv(0, u + 1, sub)

            @pl.when(jnp.logical_not(more))
            def _():
                issue_wo(sub)

            if sub == 0:
                wait_all(kbuf.at[slot], kv_sem.at[0, slot])
            for j in range(sub * hps, (sub + 1) * hps):
                qh = q_scr[h0 + j].astype(bf16)
                s = jax.lax.dot_general(qh, kbuf[slot, j], nt, preferred_element_type=f32)
                m = jnp.max(s, axis=-1, keepdims=True)
                e = jnp.exp((s - m) * scale)
                l = jnp.sum(e, axis=-1, keepdims=True)
                p_scr[j] = e * (1.0 / l)

        for sub in range(_NSUB):
            @pl.when(more)
            def _():
                issue_kv(1, u + 1, sub)

            if sub == 0:
                @pl.when(jnp.logical_not(more))
                def _():
                    issue_ffn(0, _FFN_CUT[0])

            if sub == 0:
                wait_all(vbuf.at[slot], kv_sem.at[1, slot])
            for j in range(sub * hps, (sub + 1) * hps):
                o = jnp.dot(p_scr[j].astype(bf16), vbuf[slot, j], preferred_element_type=f32)
                oh_scr[h0 + j] = jnp.where(row == b, o, oh_scr[h0 + j])
        return carry

    jax.lax.fori_loop(0, n_units, body, 0)

    issue_ffn(_FFN_CUT[0], _FFN_CUT[1])
    o_all = jnp.concatenate([oh_scr[hh] for hh in range(_HQ)], axis=-1).astype(bf16)
    wait_all(wo_buf, w_sem.at[S_O])
    attn = jnp.dot(o_all, wo_buf[...], preferred_element_type=f32)
    x1 = x + ga * attn
    h2 = (_layernorm(x1) * (1.0 + cb) + sb).astype(bf16)
    issue_ffn(_FFN_CUT[1], n_ffn)
    wait_all(wg_buf, w_sem.at[S_G])
    g = jax.lax.dot_general(h2, wg_buf[...], nt, preferred_element_type=f32)
    wait_all(wu_buf, w_sem.at[S_U])
    up = jax.lax.dot_general(h2, wu_buf[...], nt, preferred_element_type=f32)
    hid = (_sigmoid(g) * up).astype(bf16)
    out = x1
    for lo, hi, s in ((d2, F, S_D), (d1, d2, S_D1), (0, d1, S_D2)):
        wait_all(wd_buf.at[pl.ds(lo, hi - lo)], w_sem.at[s])
        out = out + gb * jnp.dot(hid[:, lo:hi], wd_buf[lo:hi, :], preferred_element_type=f32)
    o_ref[...] = out.astype(o_ref.dtype)


@jax.jit
def pallas_adaLN_cond__sliding_block_cached__glu_gated_glu__decode_kernel(
    A_x: jax.Array,
    A_k_cache: jax.Array,
    A_v_cache: jax.Array,
    A_wq: jax.Array,
    A_wo: jax.Array,
    B_x: jax.Array,
    B_w_gate: jax.Array,
    B_w_up: jax.Array,
    B_w_down: jax.Array,
    c: jax.Array,
    w_mod: jax.Array,
):
    B, Sq, D = A_x.shape
    _, Hkv, Sk, Dh = A_k_cache.shape
    F = B_w_down.shape[0]
    assert Sq == 1 and Hkv == _HQ and Dh == _DH
    W = min(4096, max(256, Sk // 4))
    bf16 = jnp.bfloat16

    hbm_spec = pl.BlockSpec(memory_space=pltpu.MemorySpace.HBM)
    out = pl.pallas_call(
        functools.partial(_kernel, B=B, D=D, F=F, Sk=Sk, W=W),
        out_shape=jax.ShapeDtypeStruct((B, D), A_x.dtype),
        in_specs=[hbm_spec] * 10,
        out_specs=pl.BlockSpec(memory_space=pltpu.VMEM),
        scratch_shapes=[
            pltpu.VMEM((2, _HU, W, _DH), bf16),
            pltpu.VMEM((2, _HU, W, _DH), bf16),
            pltpu.VMEM(A_wq.shape, bf16),
            pltpu.VMEM(A_wo.shape, bf16),
            pltpu.VMEM((F, D), bf16),
            pltpu.VMEM((F, D), bf16),
            pltpu.VMEM((F, D), bf16),
            pltpu.VMEM(w_mod.shape, bf16),
            pltpu.VMEM((B, D), bf16),
            pltpu.VMEM((B, D), bf16),
            pltpu.VMEM((_HQ, B, _DH), jnp.float32),
            pltpu.VMEM((_HU, B, W), jnp.float32),
            pltpu.VMEM((_HQ, B, _DH), jnp.float32),
            pltpu.SemaphoreType.DMA((2, 2)),
            pltpu.SemaphoreType.DMA((10,)),
        ],
        compiler_params=pltpu.CompilerParams(vmem_limit_bytes=64 * 1024 * 1024,
                                             disable_bounds_checks=True,
                                             disable_semaphore_checks=True),
    )(A_x.reshape(B, D), c, A_k_cache, A_v_cache, A_wq, A_wo, B_w_gate.T, B_w_up.T, B_w_down, w_mod)
    return out.reshape(B, Sq, D)
```

```python
import functools

import jax
import jax.numpy as jnp
import jax.experimental.pallas as pl
import jax.experimental.pallas.tpu as pltpu

_HQ = 32
_DH = 128
_HU = 16
_NHI = 2
_ROWS = 8
_NSUB = 4
_G = 4
_HSEG = 2
_FR = 32
_FSTREAM = 512
_WD_SPLIT = (128, 384)
_LO_LAG = 32
_FFN_CUT = (0.0, 0.25, 0.5, 0.75, 0.87)
_EPS = 1e-5


def _layernorm(x):
    m = jnp.mean(x, axis=-1, keepdims=True)
    xc = x - m
    v = jnp.mean(xc * xc, axis=-1, keepdims=True)
    return xc * jax.lax.rsqrt(v + _EPS)


def _sigmoid(x):
    return 1.0 / (1.0 + jnp.exp(-x))


def _kernel(x_hbm, c_hbm, k_hbm, v_hbm, wq_hbm, wo_hbm, wg_hbm, wu_hbm, wd_hbm, wmod_hbm,
            o_ref,
            kbuf, vbuf, wq_buf, wo_buf, wg_buf, wu_buf, wd_buf, wmod_buf, x_buf, c_buf,
            q_scr, p_scr, oh_scr, kv_sem, w_sem, *, B, D, F, Sk, W):
    upb = _HQ // _HU
    n_units = B * upb
    n_blk = W // _ROWS // _NSUB
    hps = _HU // _NSUB
    HD = _HQ * _DH
    f32, bf16 = jnp.float32, jnp.bfloat16
    nt = (((1,), (1,)), ((), ()))
    S_X, S_C, S_MOD, S_Q, S_O, S_G, S_U, S_D, S_D1, S_D2 = range(10)

    def copy(src, dst, sem, prio):
        pltpu.make_async_copy(src, dst, sem).start(priority=prio)

    def wait_all(buf, sem):
        pltpu.make_async_copy(buf, buf, sem).wait()

    def issue_kv(a, u, sub):
        src, dst = ((k_hbm, kbuf), (v_hbm, vbuf))[a]
        slot = u % 2
        b = u // upb
        h0 = (u % upb) * _HU

        def one(r, carry):
            r0 = pl.multiple_of((sub * n_blk + r) * _ROWS, _ROWS)
            rows_s, rows_d = pl.ds(Sk - W + r0, _ROWS), pl.ds(r0, _ROWS)
            copy(src.at[b, pl.ds(h0, _NHI), rows_s, :],
                 dst.at[slot, pl.ds(0, _NHI), rows_d, :], kv_sem.at[a, slot], 0)
            copy(src.at[b, pl.ds(h0 + _NHI, _HU - _NHI), rows_s, :],
                 dst.at[slot, pl.ds(_NHI, _HU - _NHI), rows_d, :], kv_sem.at[a, slot], 1)
            return carry

        jax.lax.fori_loop(0, n_blk, one, 0, unroll=4)

    def issue_head():
        nq = HD // D

        def one(j, carry):
            r = pl.multiple_of(j * 8, 8)
            for i in range(nq):
                cm = 6 * D // nq
                idx = (pl.ds(0, _G // 2), pl.ds(r, 8), pl.ds(i * cm, cm))
                copy(wmod_hbm.at[idx], wmod_buf.at[idx], w_sem.at[S_MOD], 0)
                for s in range(_HSEG):
                    cw = D // _HSEG
                    idx = (slice(None), pl.ds(r, 8), pl.ds(i * D + s * cw, cw))
                    copy(wq_hbm.at[idx], wq_buf.at[idx], w_sem.at[S_Q], 1)
                    if s == 0:
                        idx = (pl.ds(_G // 2, _G // 2), pl.ds(r, 8), pl.ds(i * cm, cm))
                        copy(wmod_hbm.at[idx], wmod_buf.at[idx], w_sem.at[S_MOD], 1)
                    ro = pl.multiple_of((j * nq + i) * 8, 8)
                    idx = (slice(None), pl.ds(ro, 8), pl.ds(s * cw, cw))
                    copy(wo_hbm.at[idx], wo_buf.at[idx], w_sem.at[S_O], 1)
            return carry

        jax.lax.fori_loop(0, D // _G // 8, one, 0)

    d1, d2 = _WD_SPLIT

    def rr(lo):
        starts = sorted(range(lo, F, _FR), key=lambda r: ((r - lo) % _FSTREAM, r))
        return starts

    prio4 = (0, 1, 1, 1)
    done_order = [(wg_hbm, wg_buf, S_G, r) for r in rr(0)]
    done_order += [(wu_hbm, wu_buf, S_U, r) for r in rr(0)]
    done_order += [(wd_hbm, wd_buf, S_D, r) for r in rr(d2)]
    done_order += [(wd_hbm, wd_buf, S_D1, r) for r in range(d1, d2, _FR)]
    done_order += [(wd_hbm, wd_buf, S_D2, r) for r in range(0, d1, _FR)]
    n_ffn = len(done_order)
    slots = sorted(range(n_ffn), key=lambda t: t + _LO_LAG * prio4[t % 4])
    ffn_list = [None] * n_ffn
    for piece, t in zip(done_order, slots):
        ffn_list[t] = piece
    cut = [int(f * n_ffn) for f in _FFN_CUT] + [n_ffn]

    def issue_ffn(part):
        for idx in range(cut[part], cut[part + 1]):
            src, dst, s, r = ffn_list[idx]
            rows = pl.ds(r, _FR)
            copy(src.at[rows], dst.at[rows], w_sem.at[s], prio4[idx % 4])

    issue_head()
    copy(x_hbm, x_buf, w_sem.at[S_X], 0)
    copy(c_hbm, c_buf, w_sem.at[S_C], 0)
    for sub in range(_NSUB):
        issue_kv(0, 0, sub)

    wait_all(x_buf, w_sem.at[S_X])
    wait_all(c_buf, w_sem.at[S_C])
    x = x_buf[...].astype(f32)
    c = c_buf[...].astype(f32)
    sc = (c * _sigmoid(c)).astype(bf16)
    wait_all(wmod_buf, w_sem.at[S_MOD])
    mod = jnp.dot(sc, wmod_buf[...].reshape(D, 6 * D), preferred_element_type=f32)
    sa, ca, ga, sb, cb, gb = (mod[:, i * D:(i + 1) * D] for i in range(6))
    h = (_layernorm(x) * (1.0 + ca) + sa).astype(bf16)
    issue_kv(1, 0, 0)
    wait_all(wq_buf, w_sem.at[S_Q])
    q = jnp.dot(h, wq_buf[...].reshape(D, HD), preferred_element_type=f32)
    for hh in range(_HQ):
        q_scr[hh] = q[:, hh * _DH:(hh + 1) * _DH]
    oh_scr[...] = jnp.zeros(oh_scr.shape, f32)
    for sub in range(1, _NSUB):
        issue_kv(1, 0, sub)

    scale = _DH ** -0.5
    row = jax.lax.broadcasted_iota(jnp.int32, (B, _DH), 0)

    def body(u, carry):
        slot = u % 2
        b = u // upb
        h0 = (u % upb) * _HU
        more = u + 1 < n_units

        for sub in range(_NSUB):
            @pl.when(more)
            def _():
                issue_kv(0, u + 1, sub)

            if sub * 2 % _NSUB == 0:
                @pl.when(jnp.logical_not(more))
                def _():
                    issue_ffn(sub * 2 // _NSUB)

            if sub == 0:
                wait_all(kbuf.at[slot], kv_sem.at[0, slot])
            for j in range(sub * hps, (sub + 1) * hps):
                qh = q_scr[h0 + j].astype(bf16)
                s = jax.lax.dot_general(qh, kbuf[slot, j], nt, preferred_element_type=f32)
                m = jnp.max(s, axis=-1, keepdims=True)
                e = jnp.exp((s - m) * scale)
                l = jnp.sum(e, axis=-1, keepdims=True)
                p_scr[j] = e * (1.0 / l)

        for sub in range(_NSUB):
            @pl.when(more)
            def _():
                issue_kv(1, u + 1, sub)

            if sub == 0:
                @pl.when(jnp.logical_not(more))
                def _():
                    issue_ffn(2)

                wait_all(vbuf.at[slot], kv_sem.at[1, slot])
            for j in range(sub * hps, (sub + 1) * hps):
                o = jnp.dot(p_scr[j].astype(bf16), vbuf[slot, j], preferred_element_type=f32)
                oh_scr[h0 + j] = jnp.where(row == b, o, oh_scr[h0 + j])
        return carry

    jax.lax.fori_loop(0, n_units, body, 0)

    issue_ffn(3)
    o_all = jnp.concatenate([oh_scr[hh] for hh in range(_HQ)], axis=-1).astype(bf16)
    wait_all(wo_buf, w_sem.at[S_O])
    attn = jnp.dot(o_all, wo_buf[...].reshape(HD, D), preferred_element_type=f32)
    x1 = x + ga * attn
    h2 = (_layernorm(x1) * (1.0 + cb) + sb).astype(bf16)
    issue_ffn(4)
    wait_all(wg_buf, w_sem.at[S_G])
    g = jax.lax.dot_general(h2, wg_buf[...], nt, preferred_element_type=f32)
    wait_all(wu_buf, w_sem.at[S_U])
    up = jax.lax.dot_general(h2, wu_buf[...], nt, preferred_element_type=f32)
    hid = (_sigmoid(g) * up).astype(bf16)
    out = x1
    for lo, hi, s in ((d2, F, S_D), (d1, d2, S_D1), (0, d1, S_D2)):
        wait_all(wd_buf.at[pl.ds(lo, hi - lo)], w_sem.at[s])
        out = out + gb * jnp.dot(hid[:, lo:hi], wd_buf[lo:hi, :], preferred_element_type=f32)
    o_ref[...] = out.astype(o_ref.dtype)


@jax.jit
def pallas_adaLN_cond__sliding_block_cached__glu_gated_glu__decode_kernel(
    A_x: jax.Array,
    A_k_cache: jax.Array,
    A_v_cache: jax.Array,
    A_wq: jax.Array,
    A_wo: jax.Array,
    B_x: jax.Array,
    B_w_gate: jax.Array,
    B_w_up: jax.Array,
    B_w_down: jax.Array,
    c: jax.Array,
    w_mod: jax.Array,
):
    B, Sq, D = A_x.shape
    _, Hkv, Sk, Dh = A_k_cache.shape
    F = B_w_down.shape[0]
    assert Sq == 1 and Hkv == _HQ and Dh == _DH
    W = min(4096, max(256, Sk // 4))
    bf16 = jnp.bfloat16

    def streams(w):
        return w.reshape(_G, w.shape[0] // _G, w.shape[1])

    wq, wo, wm = streams(A_wq), streams(A_wo), streams(w_mod)
    hbm_spec = pl.BlockSpec(memory_space=pltpu.MemorySpace.HBM)
    out = pl.pallas_call(
        functools.partial(_kernel, B=B, D=D, F=F, Sk=Sk, W=W),
        out_shape=jax.ShapeDtypeStruct((B, D), A_x.dtype),
        in_specs=[hbm_spec] * 10,
        out_specs=pl.BlockSpec(memory_space=pltpu.VMEM),
        scratch_shapes=[
            pltpu.VMEM((2, _HU, W, _DH), bf16),
            pltpu.VMEM((2, _HU, W, _DH), bf16),
            pltpu.VMEM(wq.shape, bf16),
            pltpu.VMEM(wo.shape, bf16),
            pltpu.VMEM((F, D), bf16),
            pltpu.VMEM((F, D), bf16),
            pltpu.VMEM((F, D), bf16),
            pltpu.VMEM(wm.shape, bf16),
            pltpu.VMEM((B, D), bf16),
            pltpu.VMEM((B, D), bf16),
            pltpu.VMEM((_HQ, B, _DH), jnp.float32),
            pltpu.VMEM((_HU, B, W), jnp.float32),
            pltpu.VMEM((_HQ, B, _DH), jnp.float32),
            pltpu.SemaphoreType.DMA((2, 2)),
            pltpu.SemaphoreType.DMA((10,)),
        ],
        compiler_params=pltpu.CompilerParams(vmem_limit_bytes=64 * 1024 * 1024,
                                             disable_bounds_checks=True,
                                             disable_semaphore_checks=True),
    )(A_x.reshape(B, D), c, A_k_cache, A_v_cache, wq, wo, B_w_gate.T, B_w_up.T, B_w_down, wm)
    return out.reshape(B, Sq, D)
```

```python
import functools

import jax
import jax.numpy as jnp
import jax.experimental.pallas as pl
import jax.experimental.pallas.tpu as pltpu

_HQ = 32
_DH = 128
_EPS = 1e-5

_HU = 16
_NHI = 2
_ROWS = 16
_NSUB = 2
_G = 4
_FR = 32
_FSTREAM = 512
_WD_SPLIT = (128, 384)
_GATE_DONE = 0.60
_UP_DONE = 0.75
_UP_LATE = 0.7
_LO_LAG = 32
_FFN_CUT = (0.0, 0.25, 0.5, 0.75, 0.87, 1.0)


def _layernorm(x):
    m = jnp.mean(x, axis=-1, keepdims=True)
    xc = x - m
    v = jnp.mean(xc * xc, axis=-1, keepdims=True)
    return xc * jax.lax.rsqrt(v + _EPS)


def _sigmoid(x):
    return 1.0 / (1.0 + jnp.exp(-x))


def _ffn_schedule(F):
    d1, d2 = _WD_SPLIT

    def interleaved(lo):
        def progress(r):
            start = lo + (r - lo) // _FSTREAM * _FSTREAM
            return (r - start + 0.5) / min(_FSTREAM, F - start)
        return sorted(range(lo, F, _FR), key=lambda r: (progress(r), r))

    def spread(m, rows, t0, t1):
        return [(t0 + (i + 0.5) * (t1 - t0) / len(rows), m, r) for i, r in enumerate(rows)]

    rg, ru, rd = interleaved(0), interleaved(0), interleaved(d2)
    n = 3 * len(rg)
    tg, tu, td = round(_GATE_DONE * n), round(_UP_DONE * n), len(rg) + len(ru) + len(rd)
    ku = len(ru) - round(_UP_LATE * (tu - tg))
    k0, k1 = tg - len(rg) - ku, tu - len(rg) - len(ru)
    t1 = td + (d2 - d1) // _FR
    plan = sorted(spread(0, rg, 0, tg)
                  + spread(1, ru[:ku], 0, tg) + spread(1, ru[ku:], tg, tu)
                  + spread(2, rd[:k0], 0, tg) + spread(2, rd[k0:k1], tg, tu) + spread(2, rd[k1:], tu, td)
                  + spread(3, range(d1, d2, _FR), td, t1) + spread(4, range(0, d1, _FR), t1, n))
    prio = [0 if t % 4 == 0 else 1 for t in range(n)]
    order = [None] * n
    for (_, m, r), t in zip(plan, sorted(range(n), key=lambda t: t + _LO_LAG * prio[t])):
        order[t] = (m, r, prio[t])
    return order


def _kernel(x_hbm, c_hbm, k_hbm, v_hbm, wq_hbm, wo_hbm, wg_hbm, wu_hbm, wd_hbm, wmod_hbm,
            o_ref,
            kbuf, vbuf, wq_buf, wo_buf, wg_buf, wu_buf, wd_buf, wmod_buf, x_buf, c_buf,
            q_scr, p_scr, oh_scr, kv_sem, w_sem, ffn_sem, *, B, D, F, Sk, W):
    upb = _HQ // _HU
    n_units = B * upb
    n_blk = W // _ROWS // _NSUB
    hps = _HU // _NSUB
    HD = _HQ * _DH
    f32, bf16 = jnp.float32, jnp.bfloat16
    nt = (((1,), (1,)), ((), ()))
    S_X, S_C, S_MOD, S_Q, S_O = range(5)

    def copy(src, dst, sem, prio):
        pltpu.make_async_copy(src, dst, sem).start(priority=prio)

    def wait_full(buf, sem):
        pltpu.make_async_copy(buf, buf, sem).wait()

    def issue_early_weights():
        nq = HD // D
        cm = 6 * D // nq
        cw = D // 2

        def one(j, carry):
            rows = pl.ds(pl.multiple_of(j * 8, 8), 8)
            for i in range(nq):
                rows_o = pl.ds(pl.multiple_of((j * nq + i) * 8, 8), 8)
                im = [(pl.ds(s * (_G // 2), _G // 2), rows, pl.ds(i * cm, cm)) for s in range(2)]
                iq = [(slice(None), rows, pl.ds(i * D + s * cw, cw)) for s in range(2)]
                io = [(slice(None), rows_o, pl.ds(s * cw, cw)) for s in range(2)]
                copy(wmod_hbm.at[im[0]], wmod_buf.at[im[0]], w_sem.at[S_MOD], 0)
                copy(wq_hbm.at[iq[0]], wq_buf.at[iq[0]], w_sem.at[S_Q], 1)
                copy(wmod_hbm.at[im[1]], wmod_buf.at[im[1]], w_sem.at[S_MOD], 1)
                copy(wo_hbm.at[io[0]], wo_buf.at[io[0]], w_sem.at[S_O], 1)
                copy(wq_hbm.at[iq[1]], wq_buf.at[iq[1]], w_sem.at[S_Q], 1)
                copy(wo_hbm.at[io[1]], wo_buf.at[io[1]], w_sem.at[S_O], 1)
            return carry

        jax.lax.fori_loop(0, D // _G // 8, one, 0)

    def issue_kv(a, u, sub):
        src, dst = ((k_hbm, kbuf), (v_hbm, vbuf))[a]
        slot = u % 2
        b = u // upb
        h0 = (u % upb) * _HU

        def one(r, carry):
            r0 = pl.multiple_of((sub * n_blk + r) * _ROWS, _ROWS)
            rows_s, rows_d = pl.ds(Sk - W + r0, _ROWS), pl.ds(r0, _ROWS)
            copy(src.at[b, pl.ds(h0, _NHI), rows_s, :],
                 dst.at[slot, pl.ds(0, _NHI), rows_d, :], kv_sem.at[a, slot], 0)
            copy(src.at[b, pl.ds(h0 + _NHI, _HU - _NHI), rows_s, :],
                 dst.at[slot, pl.ds(_NHI, _HU - _NHI), rows_d, :], kv_sem.at[a, slot], 1)
            return carry

        jax.lax.fori_loop(0, n_blk, one, 0, unroll=4)

    ffn_order = _ffn_schedule(F)
    ffn_refs = ((wg_hbm, wg_buf), (wu_hbm, wu_buf)) + ((wd_hbm, wd_buf),) * 3

    def issue_ffn(part):
        lo, hi = (int(f * len(ffn_order)) for f in _FFN_CUT[part:part + 2])
        for m, r, prio in ffn_order[lo:hi]:
            src, dst = ffn_refs[m]
            rows = pl.ds(r, _FR)
            copy(src.at[rows], dst.at[rows], ffn_sem.at[m], prio)

    issue_early_weights()
    copy(x_hbm, x_buf, w_sem.at[S_X], 0)
    copy(c_hbm, c_buf, w_sem.at[S_C], 0)
    for sub in range(_NSUB):
        issue_kv(0, 0, sub)

    wait_full(x_buf, w_sem.at[S_X])
    wait_full(c_buf, w_sem.at[S_C])
    x = x_buf[...].astype(f32)
    c = c_buf[...].astype(f32)
    sc = (c * _sigmoid(c)).astype(bf16)
    wait_full(wmod_buf, w_sem.at[S_MOD])
    mod = jnp.dot(sc, wmod_buf[...].reshape(D, 6 * D), preferred_element_type=f32)
    sa, ca, ga, sb, cb, gb = (mod[:, i * D:(i + 1) * D] for i in range(6))
    h = (_layernorm(x) * (1.0 + ca) + sa).astype(bf16)
    issue_kv(1, 0, 0)
    wait_full(wq_buf, w_sem.at[S_Q])
    q = jnp.dot(h, wq_buf[...].reshape(D, HD), preferred_element_type=f32)
    for hh in range(_HQ):
        q_scr[hh] = q[:, hh * _DH:(hh + 1) * _DH]
    oh_scr[...] = jnp.zeros(oh_scr.shape, f32)
    for sub in range(1, _NSUB):
        issue_kv(1, 0, sub)

    scale = _DH ** -0.5
    row = jax.lax.broadcasted_iota(jnp.int32, (B, _DH), 0)

    def body(u, carry):
        slot = u % 2
        b = u // upb
        h0 = (u % upb) * _HU
        more = u + 1 < n_units

        for sub in range(_NSUB):
            @pl.when(more)
            def _():
                issue_kv(0, u + 1, sub)

            if sub * 2 % _NSUB == 0:
                @pl.when(jnp.logical_not(more))
                def _():
                    issue_ffn(sub * 2 // _NSUB)

            if sub == 0:
                wait_full(kbuf.at[slot], kv_sem.at[0, slot])
            for j in range(sub * hps, (sub + 1) * hps):
                qh = q_scr[h0 + j].astype(bf16)
                s = jax.lax.dot_general(qh, kbuf[slot, j], nt, preferred_element_type=f32)
                m = jnp.max(s, axis=-1, keepdims=True)
                e = jnp.exp((s - m) * scale)
                l = jnp.sum(e, axis=-1, keepdims=True)
                p_scr[j] = e * (1.0 / l)

        for sub in range(_NSUB):
            @pl.when(more)
            def _():
                issue_kv(1, u + 1, sub)

            if sub == 0:
                @pl.when(jnp.logical_not(more))
                def _():
                    issue_ffn(2)

                wait_full(vbuf.at[slot], kv_sem.at[1, slot])
            for j in range(sub * hps, (sub + 1) * hps):
                o = jnp.dot(p_scr[j].astype(bf16), vbuf[slot, j], preferred_element_type=f32)
                oh_scr[h0 + j] = jnp.where(row == b, o, oh_scr[h0 + j])
        return carry

    jax.lax.fori_loop(0, n_units, body, 0)

    issue_ffn(3)
    o_all = jnp.concatenate([oh_scr[hh] for hh in range(_HQ)], axis=-1).astype(bf16)
    wait_full(wo_buf, w_sem.at[S_O])
    attn = jnp.dot(o_all, wo_buf[...].reshape(HD, D), preferred_element_type=f32)
    x1 = x + ga * attn
    h2 = (_layernorm(x1) * (1.0 + cb) + sb).astype(bf16)
    issue_ffn(4)
    wait_full(wg_buf, ffn_sem.at[0])
    g = jax.lax.dot_general(h2, wg_buf[...], nt, preferred_element_type=f32)
    wait_full(wu_buf, ffn_sem.at[1])
    up = jax.lax.dot_general(h2, wu_buf[...], nt, preferred_element_type=f32)
    hid = (_sigmoid(g) * up).astype(bf16)
    d1, d2 = _WD_SPLIT
    out = x1
    for m, (lo, hi) in enumerate(((d2, F), (d1, d2), (0, d1))):
        wait_full(wd_buf.at[pl.ds(lo, hi - lo)], ffn_sem.at[2 + m])
        out = out + gb * jnp.dot(hid[:, lo:hi], wd_buf[lo:hi, :], preferred_element_type=f32)
    o_ref[...] = out.astype(o_ref.dtype)


@jax.jit
def pallas_adaLN_cond__sliding_block_cached__glu_gated_glu__decode_kernel(
    A_x: jax.Array,
    A_k_cache: jax.Array,
    A_v_cache: jax.Array,
    A_wq: jax.Array,
    A_wo: jax.Array,
    B_x: jax.Array,
    B_w_gate: jax.Array,
    B_w_up: jax.Array,
    B_w_down: jax.Array,
    c: jax.Array,
    w_mod: jax.Array,
):
    B, Sq, D = A_x.shape
    _, Hkv, Sk, Dh = A_k_cache.shape
    F = B_w_down.shape[0]
    assert Sq == 1 and Hkv == _HQ and Dh == _DH and F % _FR == 0
    W = min(4096, max(256, Sk // 4))
    bf16 = jnp.bfloat16

    def streams(w):
        return w.reshape(_G, w.shape[0] // _G, w.shape[1])

    wq, wo, wm = streams(A_wq), streams(A_wo), streams(w_mod)
    hbm_spec = pl.BlockSpec(memory_space=pltpu.MemorySpace.HBM)
    out = pl.pallas_call(
        functools.partial(_kernel, B=B, D=D, F=F, Sk=Sk, W=W),
        out_shape=jax.ShapeDtypeStruct((B, D), A_x.dtype),
        in_specs=[hbm_spec] * 10,
        out_specs=pl.BlockSpec(memory_space=pltpu.VMEM),
        scratch_shapes=[
            pltpu.VMEM((2, _HU, W, _DH), bf16),
            pltpu.VMEM((2, _HU, W, _DH), bf16),
            pltpu.VMEM(wq.shape, bf16),
            pltpu.VMEM(wo.shape, bf16),
            pltpu.VMEM((F, D), bf16),
            pltpu.VMEM((F, D), bf16),
            pltpu.VMEM((F, D), bf16),
            pltpu.VMEM(wm.shape, bf16),
            pltpu.VMEM((B, D), bf16),
            pltpu.VMEM((B, D), bf16),
            pltpu.VMEM((_HQ, B, _DH), jnp.float32),
            pltpu.VMEM((_HU, B, W), jnp.float32),
            pltpu.VMEM((_HQ, B, _DH), jnp.float32),
            pltpu.SemaphoreType.DMA((2, 2)),
            pltpu.SemaphoreType.DMA((5,)),
            pltpu.SemaphoreType.DMA((5,)),
        ],
        compiler_params=pltpu.CompilerParams(vmem_limit_bytes=64 * 1024 * 1024,
                                             disable_bounds_checks=True,
                                             disable_semaphore_checks=True),
    )(A_x.reshape(B, D), c, A_k_cache, A_v_cache, wq, wo, B_w_gate.T, B_w_up.T, B_w_down, wm)
    return out.reshape(B, Sq, D)
```

```python
import functools

import jax
import jax.numpy as jnp
import jax.experimental.pallas as pl
import jax.experimental.pallas.tpu as pltpu

_HQ = 32
_DH = 128
_EPS = 1e-5

_HU = 16
_NHI = 2
_ROWS = 16
_NSUB = 2
_G = 4
_FR = 32
_FSTREAM = 512
_WD_SPLIT = (128, 384)
_GATE_DONE = 0.60
_UP_DONE = 0.75
_UP_LATE = 0.7
_LO_LAG = 32


def _layernorm(x):
    m = jnp.mean(x, axis=-1, keepdims=True)
    xc = x - m
    v = jnp.mean(xc * xc, axis=-1, keepdims=True)
    return xc * jax.lax.rsqrt(v + _EPS)


def _sigmoid(x):
    return 1.0 / (1.0 + jnp.exp(-x))


def _ffn_schedule(F):
    d1, d2 = _WD_SPLIT

    def interleaved(lo):
        def progress(r):
            start = lo + (r - lo) // _FSTREAM * _FSTREAM
            return (r - start + 0.5) / min(_FSTREAM, F - start)
        return sorted(range(lo, F, _FR), key=lambda r: (progress(r), r))

    def spread(m, rows, t0, t1):
        return [(t0 + (i + 0.5) * (t1 - t0) / len(rows), m, r) for i, r in enumerate(rows)]

    rg, ru, rd = interleaved(0), interleaved(0), interleaved(d2)
    n = 3 * len(rg)
    tg, tu, td = round(_GATE_DONE * n), round(_UP_DONE * n), len(rg) + len(ru) + len(rd)
    ku = len(ru) - round(_UP_LATE * (tu - tg))
    k0, k1 = tg - len(rg) - ku, tu - len(rg) - len(ru)
    t1 = td + (d2 - d1) // _FR
    plan = sorted(spread(0, rg, 0, tg)
                  + spread(1, ru[:ku], 0, tg) + spread(1, ru[ku:], tg, tu)
                  + spread(2, rd[:k0], 0, tg) + spread(2, rd[k0:k1], tg, tu) + spread(2, rd[k1:], tu, td)
                  + spread(3, range(d1, d2, _FR), td, t1) + spread(4, range(0, d1, _FR), t1, n))
    prio = [0 if t % 4 == 0 else 1 for t in range(n)]
    order = [None] * n
    for (_, m, r), t in zip(plan, sorted(range(n), key=lambda t: t + _LO_LAG * prio[t])):
        order[t] = (m, r, prio[t])
    return order


def _kernel(x_hbm, c_hbm, k_hbm, v_hbm, wq_hbm, wo_hbm, wg_hbm, wu_hbm, wd_hbm, wmod_hbm,
            o_ref,
            kbuf, vbuf, wq_buf, wo_buf, wg_buf, wu_buf, wd_buf, wmod_buf, x_buf, c_buf,
            q_scr, p_scr, oh_scr, kv_sem, w_sem, ffn_sem, *, B, D, F, Sk, W):
    upb = _HQ // _HU
    n_units = B * upb
    n_blk = W // _ROWS // _NSUB
    hps = _HU // _NSUB
    HD = _HQ * _DH
    f32, bf16 = jnp.float32, jnp.bfloat16
    nt = (((1,), (1,)), ((), ()))
    S_X, S_C, S_MOD, S_Q, S_O = range(5)

    def copy(src, dst, sem, prio):
        pltpu.make_async_copy(src, dst, sem).start(priority=prio)

    def wait_full(buf, sem):
        pltpu.make_async_copy(buf, buf, sem).wait()

    def issue_early_weights():
        nq = HD // D
        cm = 6 * D // nq
        cw = D // 2

        def one(j, carry):
            rows = pl.ds(pl.multiple_of(j * 8, 8), 8)
            for i in range(nq):
                rows_o = pl.ds(pl.multiple_of((j * nq + i) * 8, 8), 8)
                im = [(pl.ds(s * (_G // 2), _G // 2), rows, pl.ds(i * cm, cm)) for s in range(2)]
                iq = [(slice(None), rows, pl.ds(i * D + s * cw, cw)) for s in range(2)]
                io = [(slice(None), rows_o, pl.ds(s * cw, cw)) for s in range(2)]
                copy(wmod_hbm.at[im[0]], wmod_buf.at[im[0]], w_sem.at[S_MOD], 0)
                copy(wq_hbm.at[iq[0]], wq_buf.at[iq[0]], w_sem.at[S_Q], 1)
                copy(wmod_hbm.at[im[1]], wmod_buf.at[im[1]], w_sem.at[S_MOD], 1)
                copy(wo_hbm.at[io[0]], wo_buf.at[io[0]], w_sem.at[S_O], 1)
                copy(wq_hbm.at[iq[1]], wq_buf.at[iq[1]], w_sem.at[S_Q], 1)
                copy(wo_hbm.at[io[1]], wo_buf.at[io[1]], w_sem.at[S_O], 1)
            return carry

        jax.lax.fori_loop(0, D // _G // 8, one, 0)

    def issue_kv(a, u, sub):
        src, dst = ((k_hbm, kbuf), (v_hbm, vbuf))[a]
        slot = u % 2
        b = u // upb
        h0 = (u % upb) * _HU

        def one(r, carry):
            r0 = pl.multiple_of((sub * n_blk + r) * _ROWS, _ROWS)
            rows_s, rows_d = pl.ds(Sk - W + r0, _ROWS), pl.ds(r0, _ROWS)
            copy(src.at[b, pl.ds(h0, _NHI), rows_s, :],
                 dst.at[slot, pl.ds(0, _NHI), rows_d, :], kv_sem.at[a, slot], 0)
            copy(src.at[b, pl.ds(h0 + _NHI, _HU - _NHI), rows_s, :],
                 dst.at[slot, pl.ds(_NHI, _HU - _NHI), rows_d, :], kv_sem.at[a, slot], 1)
            return carry

        jax.lax.fori_loop(0, n_blk, one, 0, unroll=4)

    ffn_order = _ffn_schedule(F)
    ffn_refs = ((wg_hbm, wg_buf), (wu_hbm, wu_buf)) + ((wd_hbm, wd_buf),) * 3

    def issue_ffn(quarter):
        n = len(ffn_order)
        for m, r, prio in ffn_order[quarter * n // 4:(quarter + 1) * n // 4]:
            src, dst = ffn_refs[m]
            rows = pl.ds(r, _FR)
            copy(src.at[rows], dst.at[rows], ffn_sem.at[m], prio)

    issue_early_weights()
    copy(x_hbm, x_buf, w_sem.at[S_X], 0)
    copy(c_hbm, c_buf, w_sem.at[S_C], 0)
    for sub in range(_NSUB):
        issue_kv(0, 0, sub)

    wait_full(x_buf, w_sem.at[S_X])
    wait_full(c_buf, w_sem.at[S_C])
    x = x_buf[...].astype(f32)
    c = c_buf[...].astype(f32)
    sc = (c * _sigmoid(c)).astype(bf16)
    wait_full(wmod_buf, w_sem.at[S_MOD])
    mod = jnp.dot(sc, wmod_buf[...].reshape(D, 6 * D), preferred_element_type=f32)
    sa, ca, ga, sb, cb, gb = (mod[:, i * D:(i + 1) * D] for i in range(6))
    h = (_layernorm(x) * (1.0 + ca) + sa).astype(bf16)
    issue_kv(1, 0, 0)
    wait_full(wq_buf, w_sem.at[S_Q])
    wait_full(wo_buf, w_sem.at[S_O])
    q = jnp.dot(h, wq_buf[...].reshape(D, HD), preferred_element_type=f32)
    for hh in range(_HQ):
        q_scr[hh] = q[:, hh * _DH:(hh + 1) * _DH]
    oh_scr[...] = jnp.zeros(oh_scr.shape, f32)
    for sub in range(1, _NSUB):
        issue_kv(1, 0, sub)

    scale = _DH ** -0.5
    row = jax.lax.broadcasted_iota(jnp.int32, (B, _DH), 0)

    def body(u, carry):
        slot = u % 2
        b = u // upb
        h0 = (u % upb) * _HU
        more = u + 1 < n_units

        for sub in range(_NSUB):
            @pl.when(more)
            def _():
                issue_kv(0, u + 1, sub)

            if sub * 2 % _NSUB == 0:
                @pl.when(jnp.logical_not(more))
                def _():
                    issue_ffn(sub * 2 // _NSUB)

            if sub == 0:
                wait_full(kbuf.at[slot], kv_sem.at[0, slot])
            for j in range(sub * hps, (sub + 1) * hps):
                qh = q_scr[h0 + j].astype(bf16)
                s = jax.lax.dot_general(qh, kbuf[slot, j], nt, preferred_element_type=f32)
                m = jnp.max(s, axis=-1, keepdims=True)
                e = jnp.exp((s - m) * scale)
                l = jnp.sum(e, axis=-1, keepdims=True)
                p_scr[j] = e * (1.0 / l)

        for sub in range(_NSUB):
            @pl.when(more)
            def _():
                issue_kv(1, u + 1, sub)

            if sub == 0:
                @pl.when(jnp.logical_not(more))
                def _():
                    issue_ffn(2)

                wait_full(vbuf.at[slot], kv_sem.at[1, slot])
            for j in range(sub * hps, (sub + 1) * hps):
                o = jnp.dot(p_scr[j].astype(bf16), vbuf[slot, j], preferred_element_type=f32)
                oh_scr[h0 + j] = jnp.where(row == b, o, oh_scr[h0 + j])
        return carry

    jax.lax.fori_loop(0, n_units, body, 0)

    issue_ffn(3)
    o_all = jnp.concatenate([oh_scr[hh] for hh in range(_HQ)], axis=-1).astype(bf16)
    attn = jnp.dot(o_all, wo_buf[...].reshape(HD, D), preferred_element_type=f32)
    x1 = x + ga * attn
    h2 = (_layernorm(x1) * (1.0 + cb) + sb).astype(bf16)
    wait_full(wg_buf, ffn_sem.at[0])
    g = jax.lax.dot_general(h2, wg_buf[...], nt, preferred_element_type=f32)
    wait_full(wu_buf, ffn_sem.at[1])
    up = jax.lax.dot_general(h2, wu_buf[...], nt, preferred_element_type=f32)
    hid = (_sigmoid(g) * up).astype(bf16)
    d1, d2 = _WD_SPLIT
    out = x1
    for m, (lo, hi) in enumerate(((d2, F), (d1, d2), (0, d1))):
        wait_full(wd_buf.at[pl.ds(lo, hi - lo)], ffn_sem.at[2 + m])
        out = out + gb * jnp.dot(hid[:, lo:hi], wd_buf[lo:hi, :], preferred_element_type=f32)
    o_ref[...] = out.astype(o_ref.dtype)


@jax.jit
def pallas_adaLN_cond__sliding_block_cached__glu_gated_glu__decode_kernel(
    A_x: jax.Array,
    A_k_cache: jax.Array,
    A_v_cache: jax.Array,
    A_wq: jax.Array,
    A_wo: jax.Array,
    B_x: jax.Array,
    B_w_gate: jax.Array,
    B_w_up: jax.Array,
    B_w_down: jax.Array,
    c: jax.Array,
    w_mod: jax.Array,
):
    B, Sq, D = A_x.shape
    _, Hkv, Sk, Dh = A_k_cache.shape
    F = B_w_down.shape[0]
    assert Sq == 1 and Hkv == _HQ and Dh == _DH and F % _FR == 0
    W = min(4096, max(256, Sk // 4))
    bf16 = jnp.bfloat16

    def streams(w):
        return w.reshape(_G, w.shape[0] // _G, w.shape[1])

    wq, wo, wm = streams(A_wq), streams(A_wo), streams(w_mod)
    hbm_spec = pl.BlockSpec(memory_space=pltpu.MemorySpace.HBM)
    out = pl.pallas_call(
        functools.partial(_kernel, B=B, D=D, F=F, Sk=Sk, W=W),
        out_shape=jax.ShapeDtypeStruct((B, D), A_x.dtype),
        in_specs=[hbm_spec] * 10,
        out_specs=pl.BlockSpec(memory_space=pltpu.VMEM),
        scratch_shapes=[
            pltpu.VMEM((2, _HU, W, _DH), bf16),
            pltpu.VMEM((2, _HU, W, _DH), bf16),
            pltpu.VMEM(wq.shape, bf16),
            pltpu.VMEM(wo.shape, bf16),
            pltpu.VMEM((F, D), bf16),
            pltpu.VMEM((F, D), bf16),
            pltpu.VMEM((F, D), bf16),
            pltpu.VMEM(wm.shape, bf16),
            pltpu.VMEM((B, D), bf16),
            pltpu.VMEM((B, D), bf16),
            pltpu.VMEM((_HQ, B, _DH), jnp.float32),
            pltpu.VMEM((_HU, B, W), jnp.float32),
            pltpu.VMEM((_HQ, B, _DH), jnp.float32),
            pltpu.SemaphoreType.DMA((2, 2)),
            pltpu.SemaphoreType.DMA((5,)),
            pltpu.SemaphoreType.DMA((5,)),
        ],
        compiler_params=pltpu.CompilerParams(vmem_limit_bytes=64 * 1024 * 1024,
                                             disable_bounds_checks=True,
                                             disable_semaphore_checks=True),
    )(A_x.reshape(B, D), c, A_k_cache, A_v_cache, wq, wo, B_w_gate.T, B_w_up.T, B_w_down, wm)
    return out.reshape(B, Sq, D)
```

```python
import functools

import jax
import jax.numpy as jnp
import jax.experimental.pallas as pl
import jax.experimental.pallas.tpu as pltpu

_HQ = 32
_DH = 128
_EPS = 1e-5

_HU = 16
_NHI = 2
_ROWS = 16
_NSUB = 2
_G = 4
_FR = 32
_FSTREAM = 512
_WD_SPLIT = (128, 384)
_GATE_DONE = 0.60
_UP_DONE = 0.75
_UP_LATE = 0.7
_LO_LAG = 32


def _layernorm(x):
    m = jnp.mean(x, axis=-1, keepdims=True)
    xc = x - m
    v = jnp.mean(xc * xc, axis=-1, keepdims=True)
    return xc * jax.lax.rsqrt(v + _EPS)


def _sigmoid(x):
    return 1.0 / (1.0 + jnp.exp(-x))


def _ffn_schedule(F):
    d1, d2 = _WD_SPLIT

    def interleaved(lo):
        def progress(r):
            start = lo + (r - lo) // _FSTREAM * _FSTREAM
            return (r - start + 0.5) / min(_FSTREAM, F - start)
        return sorted(range(lo, F, _FR), key=lambda r: (progress(r), r))

    def spread(m, rows, t0, t1):
        return [(t0 + (i + 0.5) * (t1 - t0) / len(rows), m, r) for i, r in enumerate(rows)]

    rg, ru, rd = interleaved(0), interleaved(0), interleaved(d2)
    n = 3 * len(rg)
    tg, tu, td = round(_GATE_DONE * n), round(_UP_DONE * n), len(rg) + len(ru) + len(rd)
    ku = len(ru) - round(_UP_LATE * (tu - tg))
    k0, k1 = tg - len(rg) - ku, tu - len(rg) - len(ru)
    t1 = td + (d2 - d1) // _FR
    plan = sorted(spread(0, rg, 0, tg)
                  + spread(1, ru[:ku], 0, tg) + spread(1, ru[ku:], tg, tu)
                  + spread(2, rd[:k0], 0, tg) + spread(2, rd[k0:k1], tg, tu) + spread(2, rd[k1:], tu, td)
                  + spread(3, range(d1, d2, _FR), td, t1) + spread(4, range(0, d1, _FR), t1, n))
    prio = [0 if t % 4 == 0 else 1 for t in range(n)]
    order = [None] * n
    for (_, m, r), t in zip(plan, sorted(range(n), key=lambda t: t + _LO_LAG * prio[t])):
        order[t] = (m, r, prio[t])
    return order


def _kernel(x_hbm, c_hbm, k_hbm, v_hbm, wq_hbm, wo_hbm, wg_hbm, wu_hbm, wd_hbm, wmod_hbm,
            o_ref,
            kbuf, vbuf, wq_buf, wo_buf, wg_buf, wu_buf, wd_buf, wmod_buf, x_buf, c_buf,
            q_scr, p_scr, oh_scr, kv_sem, w_sem, ffn_sem, *, B, D, F, Sk, W):
    upb = _HQ // _HU
    n_units = B * upb
    n_blk = W // _ROWS // _NSUB
    hps = _HU // _NSUB
    HD = _HQ * _DH
    f32, bf16 = jnp.float32, jnp.bfloat16
    nt = (((1,), (1,)), ((), ()))
    S_X, S_C, S_MOD, S_Q, S_O = range(5)

    def copy(src, dst, sem, prio):
        pltpu.make_async_copy(src, dst, sem).start(priority=prio)

    def wait_full(buf, sem):
        pltpu.make_async_copy(buf, buf, sem).wait()

    def issue_early_weights():
        nq = HD // D
        cm = 6 * D // nq
        cw = D // 2

        def one(j, carry):
            rows = pl.ds(pl.multiple_of(j * 8, 8), 8)
            for i in range(nq):
                rows_o = pl.ds(pl.multiple_of((j * nq + i) * 8, 8), 8)
                im = [(pl.ds(s * (_G // 2), _G // 2), rows, pl.ds(i * cm, cm)) for s in range(2)]
                iq = [(slice(None), rows, pl.ds(i * D + s * cw, cw)) for s in range(2)]
                io = [(slice(None), rows_o, pl.ds(s * cw, cw)) for s in range(2)]
                copy(wmod_hbm.at[im[0]], wmod_buf.at[im[0]], w_sem.at[S_MOD], 0)
                copy(wq_hbm.at[iq[0]], wq_buf.at[iq[0]], w_sem.at[S_Q], 1)
                copy(wmod_hbm.at[im[1]], wmod_buf.at[im[1]], w_sem.at[S_MOD], 1)
                copy(wo_hbm.at[io[0]], wo_buf.at[io[0]], w_sem.at[S_O], 1)
                copy(wq_hbm.at[iq[1]], wq_buf.at[iq[1]], w_sem.at[S_Q], 1)
                copy(wo_hbm.at[io[1]], wo_buf.at[io[1]], w_sem.at[S_O], 1)
            return carry

        jax.lax.fori_loop(0, D // _G // 8, one, 0)

    def issue_kv(a, u, sub):
        src, dst = ((k_hbm, kbuf), (v_hbm, vbuf))[a]
        slot = u % 2
        b = u // upb
        h0 = (u % upb) * _HU

        def piece(h, n, r0, rows, prio):
            copy(src.at[b, pl.ds(h0 + h, n), pl.ds(Sk - W + r0, rows), :],
                 dst.at[slot, pl.ds(h, n), pl.ds(r0, rows), :], kv_sem.at[a, slot], prio)

        def one(r, carry):
            r0 = pl.multiple_of((sub * n_blk + r) * _ROWS, _ROWS)
            piece(0, _NHI, r0, _ROWS, 0)
            piece(_NHI, _HU - _NHI, r0, _ROWS // 2, 1)
            piece(_NHI, _HU - _NHI, r0 + _ROWS // 2, _ROWS // 2, 1)
            return carry

        jax.lax.fori_loop(0, n_blk, one, 0, unroll=2)

    ffn_order = _ffn_schedule(F)
    ffn_refs = ((wg_hbm, wg_buf), (wu_hbm, wu_buf)) + ((wd_hbm, wd_buf),) * 3

    def issue_ffn(quarter):
        n = len(ffn_order)
        for m, r, prio in ffn_order[quarter * n // 4:(quarter + 1) * n // 4]:
            src, dst = ffn_refs[m]
            rows = pl.ds(r, _FR)
            copy(src.at[rows], dst.at[rows], ffn_sem.at[m], prio)

    issue_early_weights()
    copy(x_hbm, x_buf, w_sem.at[S_X], 0)
    copy(c_hbm, c_buf, w_sem.at[S_C], 0)
    for sub in range(_NSUB):
        issue_kv(0, 0, sub)

    wait_full(x_buf, w_sem.at[S_X])
    wait_full(c_buf, w_sem.at[S_C])
    x = x_buf[...].astype(f32)
    c = c_buf[...].astype(f32)
    sc = (c * _sigmoid(c)).astype(bf16)
    wait_full(wmod_buf, w_sem.at[S_MOD])
    mod = jnp.dot(sc, wmod_buf[...].reshape(D, 6 * D), preferred_element_type=f32)
    sa, ca, ga, sb, cb, gb = (mod[:, i * D:(i + 1) * D] for i in range(6))
    h = (_layernorm(x) * (1.0 + ca) + sa).astype(bf16)
    issue_kv(1, 0, 0)
    wait_full(wq_buf, w_sem.at[S_Q])
    wait_full(wo_buf, w_sem.at[S_O])
    q = jnp.dot(h, wq_buf[...].reshape(D, HD), preferred_element_type=f32)
    for hh in range(_HQ):
        q_scr[hh] = q[:, hh * _DH:(hh + 1) * _DH]
    oh_scr[...] = jnp.zeros(oh_scr.shape, f32)
    for sub in range(1, _NSUB):
        issue_kv(1, 0, sub)

    scale = _DH ** -0.5
    row = jax.lax.broadcasted_iota(jnp.int32, (B, _DH), 0)

    def body(u, carry):
        slot = u % 2
        b = u // upb
        h0 = (u % upb) * _HU
        more = u + 1 < n_units

        for sub in range(_NSUB):
            @pl.when(more)
            def _():
                issue_kv(0, u + 1, sub)

            if sub * 2 % _NSUB == 0:
                @pl.when(jnp.logical_not(more))
                def _():
                    issue_ffn(sub * 2 // _NSUB)

            if sub == 0:
                wait_full(kbuf.at[slot], kv_sem.at[0, slot])
            for j in range(sub * hps, (sub + 1) * hps):
                qh = q_scr[h0 + j].astype(bf16)
                s = jax.lax.dot_general(qh, kbuf[slot, j], nt, preferred_element_type=f32)
                m = jnp.max(s, axis=-1, keepdims=True)
                e = jnp.exp((s - m) * scale)
                l = jnp.sum(e, axis=-1, keepdims=True)
                p_scr[j] = e * (1.0 / l)

        for sub in range(_NSUB):
            @pl.when(more)
            def _():
                issue_kv(1, u + 1, sub)

            if sub == 0:
                @pl.when(jnp.logical_not(more))
                def _():
                    issue_ffn(2)

                wait_full(vbuf.at[slot], kv_sem.at[1, slot])
            for j in range(sub * hps, (sub + 1) * hps):
                o = jnp.dot(p_scr[j].astype(bf16), vbuf[slot, j], preferred_element_type=f32)
                oh_scr[h0 + j] = jnp.where(row == b, o, oh_scr[h0 + j])
        return carry

    jax.lax.fori_loop(0, n_units, body, 0)

    issue_ffn(3)
    o_all = jnp.concatenate([oh_scr[hh] for hh in range(_HQ)], axis=-1).astype(bf16)
    attn = jnp.dot(o_all, wo_buf[...].reshape(HD, D), preferred_element_type=f32)
    x1 = x + ga * attn
    h2 = (_layernorm(x1) * (1.0 + cb) + sb).astype(bf16)
    wait_full(wg_buf, ffn_sem.at[0])
    g = jax.lax.dot_general(h2, wg_buf[...], nt, preferred_element_type=f32)
    wait_full(wu_buf, ffn_sem.at[1])
    up = jax.lax.dot_general(h2, wu_buf[...], nt, preferred_element_type=f32)
    hid = (_sigmoid(g) * up).astype(bf16)
    d1, d2 = _WD_SPLIT
    out = x1
    for m, (lo, hi) in enumerate(((d2, F), (d1, d2), (0, d1))):
        wait_full(wd_buf.at[pl.ds(lo, hi - lo)], ffn_sem.at[2 + m])
        out = out + gb * jnp.dot(hid[:, lo:hi], wd_buf[lo:hi, :], preferred_element_type=f32)
    o_ref[...] = out.astype(o_ref.dtype)


@jax.jit
def pallas_adaLN_cond__sliding_block_cached__glu_gated_glu__decode_kernel(
    A_x: jax.Array,
    A_k_cache: jax.Array,
    A_v_cache: jax.Array,
    A_wq: jax.Array,
    A_wo: jax.Array,
    B_x: jax.Array,
    B_w_gate: jax.Array,
    B_w_up: jax.Array,
    B_w_down: jax.Array,
    c: jax.Array,
    w_mod: jax.Array,
):
    B, Sq, D = A_x.shape
    _, Hkv, Sk, Dh = A_k_cache.shape
    F = B_w_down.shape[0]
    assert Sq == 1 and Hkv == _HQ and Dh == _DH and F % _FR == 0
    W = min(4096, max(256, Sk // 4))
    bf16 = jnp.bfloat16

    def streams(w):
        return w.reshape(_G, w.shape[0] // _G, w.shape[1])

    wq, wo, wm = streams(A_wq), streams(A_wo), streams(w_mod)
    hbm_spec = pl.BlockSpec(memory_space=pltpu.MemorySpace.HBM)
    out = pl.pallas_call(
        functools.partial(_kernel, B=B, D=D, F=F, Sk=Sk, W=W),
        out_shape=jax.ShapeDtypeStruct((B, D), A_x.dtype),
        in_specs=[hbm_spec] * 10,
        out_specs=pl.BlockSpec(memory_space=pltpu.VMEM),
        scratch_shapes=[
            pltpu.VMEM((2, _HU, W, _DH), bf16),
            pltpu.VMEM((2, _HU, W, _DH), bf16),
            pltpu.VMEM(wq.shape, bf16),
            pltpu.VMEM(wo.shape, bf16),
            pltpu.VMEM((F, D), bf16),
            pltpu.VMEM((F, D), bf16),
            pltpu.VMEM((F, D), bf16),
            pltpu.VMEM(wm.shape, bf16),
            pltpu.VMEM((B, D), bf16),
            pltpu.VMEM((B, D), bf16),
            pltpu.VMEM((_HQ, B, _DH), jnp.float32),
            pltpu.VMEM((_HU, B, W), jnp.float32),
            pltpu.VMEM((_HQ, B, _DH), jnp.float32),
            pltpu.SemaphoreType.DMA((2, 2)),
            pltpu.SemaphoreType.DMA((5,)),
            pltpu.SemaphoreType.DMA((5,)),
        ],
        compiler_params=pltpu.CompilerParams(vmem_limit_bytes=64 * 1024 * 1024,
                                             disable_bounds_checks=True,
                                             disable_semaphore_checks=True),
    )(A_x.reshape(B, D), c, A_k_cache, A_v_cache, wq, wo, B_w_gate.T, B_w_up.T, B_w_down, wm)
    return out.reshape(B, Sq, D)
```

```python
import functools

import jax
import jax.numpy as jnp
import jax.experimental.pallas as pl
import jax.experimental.pallas.tpu as pltpu

_HQ = 32
_DH = 128
_EPS = 1e-5

_HU = 16
_NHI = 2
_ROWS = 16
_NSUB = 2
_G = 4
_FR = 32
_FHR = 16
_FSTREAM = 512
_FSHIFT = 8
_WD_SPLIT = (128, 384)


def _layernorm(x):
    m = jnp.mean(x, axis=-1, keepdims=True)
    xc = x - m
    v = jnp.mean(xc * xc, axis=-1, keepdims=True)
    return xc * jax.lax.rsqrt(v + _EPS)


def _sigmoid(x):
    return 1.0 / (1.0 + jnp.exp(-x))


def _ffn_schedule(F):
    def cut(m, lo, hi, step):
        b = sorted({lo, hi} | {r for r in range(_FSHIFT % step, hi, step) if r > lo})
        return [(m, r0, r1 - r0) for r0, r1 in zip(b, b[1:])]

    def merge(*lists):
        ev = sorted(((j + 0.5) / len(l), i, j) for i, l in enumerate(lists) for j in range(len(l)))
        return [lists[i][j] for _, i, j in ev]

    d1, d2 = _WD_SPLIT
    s1, s2 = _FSTREAM + _FSHIFT, 2 * _FSTREAM + _FSHIFT
    dh = F - 2 * _FR + _FSHIFT
    hi = cut(0, s2, F, _FHR) + cut(1, s2, F, _FHR) + cut(2, dh, F, _FHR)
    lg = merge(cut(0, 0, s1, _FR), cut(0, s1, s2, _FR))
    lu = merge(cut(1, 0, s1, _FR), cut(1, s1, s2, _FR))
    ld = merge(cut(2, d2, d2 + s1, _FR), cut(2, d2 + s1, dh, _FR))
    ku, k0, k1 = round(0.7 * len(lu)), round(0.16 * len(ld)), round(0.4 * len(ld))
    lo = (merge(lg, lu[:ku], ld[:k0]) + merge(lu[ku:], ld[k0:k1]) + ld[k1:]
          + cut(3, d1, d2, _FR) + cut(4, 0, d1, _FR))
    return merge([p + (0,) for p in hi], [p + (1,) for p in lo])


def _kernel(x_hbm, c_hbm, k_hbm, v_hbm, wq_hbm, wo_hbm, wg_hbm, wu_hbm, wd_hbm, wmod_hbm,
            o_ref,
            kbuf, vbuf, wq_buf, wo_buf, wg_buf, wu_buf, wd_buf, wmod_buf, x_buf, c_buf,
            q_scr, p_scr, oh_scr, kv_sem, w_sem, ffn_sem, *, B, D, F, Sk, W):
    upb = _HQ // _HU
    n_units = B * upb
    n_blk = W // _ROWS // _NSUB
    hps = _HU // _NSUB
    HD = _HQ * _DH
    f32, bf16 = jnp.float32, jnp.bfloat16
    nt = (((1,), (1,)), ((), ()))
    S_X, S_C, S_MOD, S_Q, S_O = range(5)

    def copy(src, dst, sem, prio):
        pltpu.make_async_copy(src, dst, sem).start(priority=prio)

    def wait_full(buf, sem):
        pltpu.make_async_copy(buf, buf, sem).wait()

    def issue_early_weights():
        nq = HD // D
        cm = 6 * D // nq
        cw = D // 2

        def one(j, carry):
            rows = pl.ds(pl.multiple_of(j * 8, 8), 8)
            for i in range(nq):
                rows_o = pl.ds(pl.multiple_of((j * nq + i) * 8, 8), 8)
                im = [(pl.ds(s * (_G // 2), _G // 2), rows, pl.ds(i * cm, cm)) for s in range(2)]
                iq = [(slice(None), rows, pl.ds(i * D + s * cw, cw)) for s in range(2)]
                io = [(slice(None), rows_o, pl.ds(s * cw, cw)) for s in range(2)]
                copy(wmod_hbm.at[im[0]], wmod_buf.at[im[0]], w_sem.at[S_MOD], 0)
                copy(wq_hbm.at[iq[0]], wq_buf.at[iq[0]], w_sem.at[S_Q], 1)
                copy(wmod_hbm.at[im[1]], wmod_buf.at[im[1]], w_sem.at[S_MOD], 1)
                copy(wo_hbm.at[io[0]], wo_buf.at[io[0]], w_sem.at[S_O], 1)
                copy(wq_hbm.at[iq[1]], wq_buf.at[iq[1]], w_sem.at[S_Q], 1)
                copy(wo_hbm.at[io[1]], wo_buf.at[io[1]], w_sem.at[S_O], 1)
            return carry

        jax.lax.fori_loop(0, D // _G // 8, one, 0)

    def issue_kv(a, u, sub):
        src, dst = ((k_hbm, kbuf), (v_hbm, vbuf))[a]
        slot = u % 2
        b = u // upb
        h0 = (u % upb) * _HU

        def piece(h, n, r0, rows, prio):
            copy(src.at[b, pl.ds(h0 + h, n), pl.ds(Sk - W + r0, rows), :],
                 dst.at[slot, pl.ds(h, n), pl.ds(r0, rows), :], kv_sem.at[a, slot], prio)

        def one(r, carry):
            r0 = pl.multiple_of((sub * n_blk + r) * _ROWS, _ROWS)
            piece(0, _NHI, r0, _ROWS, 0)
            piece(_NHI, _HU - _NHI, r0, _ROWS // 2, 1)
            piece(_NHI, _HU - _NHI, r0 + _ROWS // 2, _ROWS // 2, 1)
            return carry

        jax.lax.fori_loop(0, n_blk, one, 0, unroll=2)

    ffn_order = _ffn_schedule(F)
    ffn_refs = ((wg_hbm, wg_buf), (wu_hbm, wu_buf)) + ((wd_hbm, wd_buf),) * 3

    def issue_ffn(quarter):
        n = len(ffn_order)
        for m, r, nr, prio in ffn_order[quarter * n // 4:(quarter + 1) * n // 4]:
            src, dst = ffn_refs[m]
            rows = pl.ds(r, nr)
            copy(src.at[rows], dst.at[rows], ffn_sem.at[m], prio)

    issue_early_weights()
    copy(x_hbm, x_buf, w_sem.at[S_X], 0)
    copy(c_hbm, c_buf, w_sem.at[S_C], 0)
    for sub in range(_NSUB):
        issue_kv(0, 0, sub)

    wait_full(x_buf, w_sem.at[S_X])
    wait_full(c_buf, w_sem.at[S_C])
    x = x_buf[...].astype(f32)
    c = c_buf[...].astype(f32)
    sc = (c * _sigmoid(c)).astype(bf16)
    wait_full(wmod_buf, w_sem.at[S_MOD])
    mod = jnp.dot(sc, wmod_buf[...].reshape(D, 6 * D), preferred_element_type=f32)
    sa, ca, ga, sb, cb, gb = (mod[:, i * D:(i + 1) * D] for i in range(6))
    h = (_layernorm(x) * (1.0 + ca) + sa).astype(bf16)
    issue_kv(1, 0, 0)
    wait_full(wq_buf, w_sem.at[S_Q])
    wait_full(wo_buf, w_sem.at[S_O])
    q = jnp.dot(h, wq_buf[...].reshape(D, HD), preferred_element_type=f32)
    for hh in range(_HQ):
        q_scr[hh] = q[:, hh * _DH:(hh + 1) * _DH]
    oh_scr[...] = jnp.zeros(oh_scr.shape, f32)
    for sub in range(1, _NSUB):
        issue_kv(1, 0, sub)

    scale = _DH ** -0.5
    row = jax.lax.broadcasted_iota(jnp.int32, (B, _DH), 0)

    def body(u, carry):
        slot = u % 2
        b = u // upb
        h0 = (u % upb) * _HU
        more = u + 1 < n_units

        for sub in range(_NSUB):
            @pl.when(more)
            def _():
                issue_kv(0, u + 1, sub)

            if sub * 2 % _NSUB == 0:
                @pl.when(jnp.logical_not(more))
                def _():
                    issue_ffn(sub * 2 // _NSUB)

            if sub == 0:
                wait_full(kbuf.at[slot], kv_sem.at[0, slot])
            for j in range(sub * hps, (sub + 1) * hps):
                qh = q_scr[h0 + j].astype(bf16)
                s = jax.lax.dot_general(qh, kbuf[slot, j], nt, preferred_element_type=f32)
                m = jnp.max(s, axis=-1, keepdims=True)
                e = jnp.exp((s - m) * scale)
                l = jnp.sum(e, axis=-1, keepdims=True)
                p_scr[j] = e * (1.0 / l)

        for sub in range(_NSUB):
            @pl.when(more)
            def _():
                issue_kv(1, u + 1, sub)

            if sub == 0:
                @pl.when(jnp.logical_not(more))
                def _():
                    issue_ffn(2)

                wait_full(vbuf.at[slot], kv_sem.at[1, slot])
            for j in range(sub * hps, (sub + 1) * hps):
                o = jnp.dot(p_scr[j].astype(bf16), vbuf[slot, j], preferred_element_type=f32)
                oh_scr[h0 + j] = jnp.where(row == b, o, oh_scr[h0 + j])
        return carry

    jax.lax.fori_loop(0, n_units, body, 0)

    issue_ffn(3)
    o_all = jnp.concatenate([oh_scr[hh] for hh in range(_HQ)], axis=-1).astype(bf16)
    attn = jnp.dot(o_all, wo_buf[...].reshape(HD, D), preferred_element_type=f32)
    x1 = x + ga * attn
    h2 = (_layernorm(x1) * (1.0 + cb) + sb).astype(bf16)
    wait_full(wg_buf, ffn_sem.at[0])
    g = jax.lax.dot_general(h2, wg_buf[...], nt, preferred_element_type=f32)
    wait_full(wu_buf, ffn_sem.at[1])
    up = jax.lax.dot_general(h2, wu_buf[...], nt, preferred_element_type=f32)
    hid = (_sigmoid(g) * up).astype(bf16)
    d1, d2 = _WD_SPLIT
    out = x1
    for m, (lo, hi) in enumerate(((d2, F), (d1, d2), (0, d1))):
        wait_full(wd_buf.at[pl.ds(lo, hi - lo)], ffn_sem.at[2 + m])
        out = out + gb * jnp.dot(hid[:, lo:hi], wd_buf[lo:hi, :], preferred_element_type=f32)
    o_ref[...] = out.astype(o_ref.dtype)


@jax.jit
def pallas_adaLN_cond__sliding_block_cached__glu_gated_glu__decode_kernel(
    A_x: jax.Array,
    A_k_cache: jax.Array,
    A_v_cache: jax.Array,
    A_wq: jax.Array,
    A_wo: jax.Array,
    B_x: jax.Array,
    B_w_gate: jax.Array,
    B_w_up: jax.Array,
    B_w_down: jax.Array,
    c: jax.Array,
    w_mod: jax.Array,
):
    B, Sq, D = A_x.shape
    _, Hkv, Sk, Dh = A_k_cache.shape
    F = B_w_down.shape[0]
    assert Sq == 1 and Hkv == _HQ and Dh == _DH
    assert F % _FR == 0 and F > 2 * (_FSTREAM + _FR)
    W = min(4096, max(256, Sk // 4))
    bf16 = jnp.bfloat16

    def streams(w):
        return w.reshape(_G, w.shape[0] // _G, w.shape[1])

    wq, wo, wm = streams(A_wq), streams(A_wo), streams(w_mod)
    hbm_spec = pl.BlockSpec(memory_space=pltpu.MemorySpace.HBM)
    out = pl.pallas_call(
        functools.partial(_kernel, B=B, D=D, F=F, Sk=Sk, W=W),
        out_shape=jax.ShapeDtypeStruct((B, D), A_x.dtype),
        in_specs=[hbm_spec] * 10,
        out_specs=pl.BlockSpec(memory_space=pltpu.VMEM),
        scratch_shapes=[
            pltpu.VMEM((2, _HU, W, _DH), bf16),
            pltpu.VMEM((2, _HU, W, _DH), bf16),
            pltpu.VMEM(wq.shape, bf16),
            pltpu.VMEM(wo.shape, bf16),
            pltpu.VMEM((F, D), bf16),
            pltpu.VMEM((F, D), bf16),
            pltpu.VMEM((F, D), bf16),
            pltpu.VMEM(wm.shape, bf16),
            pltpu.VMEM((B, D), bf16),
            pltpu.VMEM((B, D), bf16),
            pltpu.VMEM((_HQ, B, _DH), jnp.float32),
            pltpu.VMEM((_HU, B, W), jnp.float32),
            pltpu.VMEM((_HQ, B, _DH), jnp.float32),
            pltpu.SemaphoreType.DMA((2, 2)),
            pltpu.SemaphoreType.DMA((5,)),
            pltpu.SemaphoreType.DMA((5,)),
        ],
        compiler_params=pltpu.CompilerParams(vmem_limit_bytes=64 * 1024 * 1024,
                                             disable_bounds_checks=True,
                                             disable_semaphore_checks=True),
    )(A_x.reshape(B, D), c, A_k_cache, A_v_cache, wq, wo, B_w_gate.T, B_w_up.T, B_w_down, wm)
    return out.reshape(B, Sq, D)
```
